```python
import os as _os
_os.environ.setdefault("JAX_PLATFORMS", "cpu")
import jax
import jax.numpy as jnp

def _softmax(x, axis=-1):
    return jax.nn.softmax(x, axis=axis)
def _gelu(x):
    return jax.nn.gelu(x, approximate=True)
def _silu(x):
    return jax.nn.silu(x)
def _sigmoid(x):
    return jax.nn.sigmoid(x)
def _layernorm(x, axis=-1, eps=1e-5):
    m = jnp.mean(x, axis=axis, keepdims=True)
    v = jnp.var(x, axis=axis, keepdims=True)
    return (x - m) / jnp.sqrt(v + eps)
def _scatter_add(tgt, idx, src, axis=0):
    return tgt.at[idx].add(src)
def _segment_sum(src, seg, n):
    return jax.ops.segment_sum(src, seg, n)
class _Rng:
    def __init__(self, key):
        self._k = key
    def _next(self):
        self._k, sub = jax.random.split(self._k)
        return sub
    def normal(self, shape):
        return jax.random.normal(self._next(), shape, dtype=jnp.bfloat16)
    def randint(self, lo, hi, shape):
        return jax.random.randint(self._next(), shape, lo, hi, dtype=jnp.int32)
    def uniform(self, shape, lo=0.0, hi=1.0):
        return jax.random.uniform(self._next(), shape, jnp.bfloat16, lo, hi)
    def permutation(self, n):
        return jax.random.permutation(self._next(), n)


kernel_name = 'concat_heads__sliding_block__grouped_kv_mqa__prompt'

def setup_inputs():
    _rng = _Rng(jax.random.key(int.from_bytes(__import__("os").urandom(4), "little")))
    _w = (lambda a: (lambda t: t.astype(jnp.bfloat16) if jnp.issubdtype(t.dtype, jnp.floating) else t)(jnp.asarray(a)))
    def _A_setup():
        B, S, D = 1, 2048, 576
        return {
            "x": _w((lambda *s: _rng.normal(s) * 0.2)(B, S, D)),
            "wqkv": _w((lambda *s: _rng.normal(s) * 0.2)(D, 3 * D)),
            "wo": _w((lambda *s: _rng.normal(s) * 0.05)(D, D)),
        }
    _A_in = _A_setup()

    def _B_setup():
        B, S, D, H = 1, 2048, 576, 32
        Dh = D // H
        return {
            "x": _w((lambda *s: _rng.normal(s) * 0.05)(B, S, D)),
            "wq": _w((lambda *s: _rng.normal(s) * 1.6)(D, H * Dh)),
            "wk": _w((lambda *s: _rng.normal(s) * 1.6)(D, Dh)),
            "wv": _w((lambda *s: _rng.normal(s) * 0.1)(D, Dh)),
            "wo": _w((lambda *s: _rng.normal(s) * 0.1)(H * Dh, D)),
        }
    _B_in = _B_setup()

    return {
        "A_x": _A_in["x"],
        "A_wqkv": _A_in["wqkv"],
        "A_wo": _A_in["wo"],
        "B_x": _B_in["x"],
        "B_wq": _B_in["wq"],
        "B_wk": _B_in["wk"],
        "B_wv": _B_in["wv"],
        "B_wo": _B_in["wo"],
    }

def reference(A_x, A_wqkv, A_wo, B_x, B_wq, B_wk, B_wv, B_wo):
    def _A_ref(x, wqkv, wo):
        B, S, D = x.shape
        H = 32; Dh = D // H; W = 256
        qkv = (lambda x, *d: x.transpose(*d))((x @ wqkv).reshape(B, S, 3, H, Dh), 2, 0, 3, 1, 4)
        q, k, v = qkv[0], qkv[1], qkv[2]
        scores = jnp.einsum("bhqd,bhkd->bhqk", q, k) * (Dh ** -0.5)
        idx = jnp.arange(S)
        mask = (idx[:, None] - idx[None, :] >= 0) & (idx[:, None] - idx[None, :] < W)
        scores = jnp.where(mask[None, None], scores, -1e9)
        p = _softmax(scores, axis=-1)
        o = jnp.einsum("bhqk,bhkd->bhqd", p, v)
        return (lambda x, *d: x.transpose(*d))(o, 0, 2, 1, 3).reshape(B, S, D) @ wo

    def _B_ref(x, wq, wk, wv, wo):
        B, S, D = x.shape
        H = 32
        Dh = D // H
        q = (lambda x, *d: x.transpose(*d))((x @ wq).reshape(B, S, H, Dh), 0, 2, 1, 3)
        k = x @ wk
        v = x @ wv
        scores = jnp.einsum("bhqd,bkd->bhqk", q, k) * (Dh ** -0.5)
        p = _softmax(scores, axis=-1)
        o = jnp.einsum("bhqk,bkd->bhqd", p, v)
        return (lambda x, *d: x.transpose(*d))(o, 0, 2, 1, 3).reshape(B, S, H * Dh) @ wo

    a = _A_ref(A_x, A_wqkv, A_wo)
    b = _B_ref(B_x, B_wq, B_wk, B_wv, B_wo)
    return jnp.concatenate([a, b], axis=-1)
```

```python
import math

import jax
import jax.numpy as jnp
from jax import lax
import jax.experimental.pallas as pl
import jax.experimental.pallas.tpu as pltpu


S, D, H, DH, WIN = 2048, 576, 32, 18, 256
G = 8
GR = 4 * DH
TB = 512
F32 = jnp.float32
BF16 = jnp.bfloat16
I32 = jnp.int32
SCALE2 = (DH ** -0.5) * math.log2(math.e)
MARGIN = 1.0 + 2.0 ** -6
L_SAFE = 2.0 ** -64

NN = ((1,), (0,))


def mm(a, b):
    return lax.dot_general(a, b, (NN, ((), ())), preferred_element_type=F32)


def iota(shape, dim):
    return lax.broadcasted_iota(I32, shape, dim)


def unsafe_flag(l):
    return jnp.where(l >= L_SAFE, 0.0, 1.0)


def kernel(xa_h, wqkv_h, woa_h, xb_h, wq_h, wk_h, wv_h, wob_h, out_h,
           xa, xb, wqkv, woa, wq, wk, wv, wob,
           wbt_s, wat_s, wot_s, kb_s, vtb_s, wb_s, p0_s, ob_s,
           ka_s, vta_s, qa_s, na_s, oa_s, out_v, sems, xsem, osem):
    NTB = S // TB
    def cp(src, dst, sem):
        c = pltpu.make_async_copy(src, dst, sem)
        c.start()
        return c
    cp_wk = cp(wk_h, wk, sems.at[0])
    cp_wv = cp(wv_h, wv, sems.at[1])
    cp_wq = cp(wq_h, wq, sems.at[2])
    cp_xb = [cp(xb_h.at[:, pl.ds(tb * TB, TB)], xb.at[:, pl.ds(tb * TB, TB)], xsem.at[tb]) for tb in range(NTB)]
    cp_wqkv = cp(wqkv_h, wqkv, sems.at[3])
    cp_xa = cp(xa_h, xa, sems.at[4])
    cp_woa = cp(woa_h, woa, sems.at[5])
    cp_wob = cp(wob_h, wob, sems.at[6])

    seg = ((iota((H, D), 1) >= DH * iota((H, D), 0)) & (iota((H, D), 1) < DH * iota((H, D), 0) + DH)).astype(BF16)

    wbt_s[D:D + 64, :] = jnp.zeros((64, D), BF16)
    cp_wk.wait()
    wbt_s[D:D + DH, :] = wk[...]
    cp_wv.wait()
    wbt_s[D + 32:D + 32 + DH, :] = wv[...]
    cp_wq.wait()
    wbt_s[0:D, :] = wq[...].T

    def b_dot(tb):
        cp_xb[tb].wait()
        return mm(wbt_s[...], xb[:, tb * TB:(tb + 1) * TB])

    def b_post(tb, y, kmax):
        t0 = tb * TB
        kt = y[D:D + 32].astype(BF16).astype(F32)
        vt = y[D + 32:D + 32 + 24].astype(BF16).astype(F32)
        kb_s[t0:t0 + TB, :] = kt.T.astype(BF16)
        vtb_s[:, t0:t0 + TB] = jnp.where(iota((24, TB), 0) == DH, 1.0, vt)
        kmax = jnp.maximum(kmax, jnp.sum(kt * kt, axis=0, keepdims=True))
        q = (y[0:D] * SCALE2).astype(BF16).astype(F32)
        nq2 = mm(seg, (q * q).astype(BF16))
        c = -jnp.sqrt(nq2) * MARGIN
        r = iota((32, TB), 0)
        for h in range(H):
            a = (DH * h) // 16 * 16
            off = DH * h - a
            x = q[a:a + 32]
            if off:
                x = pltpu.roll(x, 32 - off, 0)
            w = jnp.where(r < DH, x, jnp.where(r == DH, c[h:h + 1], 0.0))
            wb_s[h, :, t0:t0 + TB] = w.astype(BF16)
        return kmax

    kmax = jnp.zeros((1, TB), F32)
    ys = {0: b_dot(0)}
    for tb in range(NTB):
        if tb + 1 < NTB:
            ys[tb + 1] = b_dot(tb + 1)
        if tb == 2:
            cp_wqkv.wait()
            wat_s[0:896, :] = wqkv[:, 0:896].T
        if tb == 3:
            wat_s[896:3 * D, :] = wqkv[:, 896:3 * D].T
        kmax = b_post(tb, ys.pop(tb), kmax)
    kn = jnp.sqrt(jnp.max(kmax, axis=1, keepdims=True)) * MARGIN
    kb_s[...] = jnp.where(iota((S, 32), 1) == DH, kn.astype(BF16), kb_s[...])

    QB = 512
    KB = 128
    NS = 1024
    NIT = G * (S // QB)

    def b_w(i):
        g = i // (S // QB)
        q0 = pl.multiple_of((i % (S // QB)) * QB, QB)
        return jnp.concatenate([wb_s[4 * g + j, :, pl.ds(q0, QB)] for j in range(4)], axis=1)

    def b_store(g, q0, nq, acc):
        l = acc[DH:DH + 1, :]
        o = jnp.concatenate([acc * (1.0 / l), jnp.zeros((8, 4 * nq), F32)], axis=0)
        r = iota((32, nq), 0)
        rows = [None] * 10
        for j in range(4):
            oj = jnp.where(r < DH, o[:, j * nq:(j + 1) * nq], 0.0)
            if j:
                oj = pltpu.roll(oj, 2 * j, 0)
            for u in range(4):
                piece = oj[8 * u:8 * u + 8]
                idx = 2 * j + u
                rows[idx] = piece if rows[idx] is None else rows[idx] + piece
        ob_s[pl.ds(pl.multiple_of(g * GR, 8), GR), pl.ds(q0, nq)] = jnp.concatenate(rows[0:9], axis=0)
        return l

    units = [(c, n) for c in range(S // KB) for n in range(4 * QB // NS)]
    p0_s[...] = jnp.exp2(mm(kb_s[0:KB, :], b_w(0)[:, 0:NS])).astype(BF16)

    def b_attn(i, bad):
        g = i // (S // QB)
        q0 = pl.multiple_of((i % (S // QB)) * QB, QB)
        w = b_w(i)
        accs = [None] * (4 * QB // NS)

        def qk(u, w):
            c, n = u
            return jnp.exp2(mm(kb_s[c * KB:(c + 1) * KB, :], w[:, n * NS:(n + 1) * NS])).astype(BF16)

        ps = {0: p0_s[...]}
        for k, (c, n) in enumerate(units):
            if k + 1 < len(units):
                ps[k + 1] = qk(units[k + 1], w)
            else:
                pn = qk(units[0], b_w(jnp.minimum(i + 1, NIT - 1)))
            r = mm(vtb_s[:, c * KB:(c + 1) * KB], ps.pop(k))
            accs[n] = r if accs[n] is None else accs[n] + r
        p0_s[...] = pn
        l = b_store(g, q0, QB, jnp.concatenate(accs, axis=1))
        for j in range(4):
            bad = jnp.maximum(bad, unsafe_flag(l[:, j * QB:(j + 1) * QB]))
        return bad
    bad_b = lax.fori_loop(0, NIT, b_attn, jnp.zeros((1, QB), F32))

    @pl.when(jnp.max(bad_b) > 0.0)
    def _b_exact():
        def body(i, carry):
            g = i // (S // 128)
            q0 = pl.multiple_of((i % (S // 128)) * 128, 128)
            accs = []
            for j in range(4):
                w = wb_s[4 * g + j, :, pl.ds(q0, 128)]
                w = jnp.where(iota((32, 128), 0) == DH, jnp.zeros_like(w), w)

                def scores(c):
                    return mm(kb_s[pl.ds(pl.multiple_of(c * 512, 512), 512), :], w)

                def max_step(c, m):
                    return jnp.maximum(m, jnp.max(scores(c), axis=0, keepdims=True))
                m = lax.fori_loop(0, S // 512, max_step, jnp.full((1, 128), -jnp.inf, F32))

                def acc_step(c, acc):
                    p = jnp.exp2(scores(c) - m).astype(BF16)
                    return acc + mm(vtb_s[:, pl.ds(pl.multiple_of(c * 512, 512), 512)], p)
                accs.append(lax.fori_loop(0, S // 512, acc_step, jnp.zeros((24, 128), F32)))
            b_store(g, q0, 128, jnp.concatenate(accs, axis=1))
            return carry
        lax.fori_loop(0, G * (S // 128), body, 0)

    cp_xa.wait()

    def a_dot(tb):
        return mm(wat_s[...], xa[:, tb * TB:(tb + 1) * TB])

    def a_post(tb, y, kmax):
        t0 = tb * TB
        yb = y.astype(BF16).astype(F32)
        q = (y[0:D + 8] * SCALE2).astype(BF16).astype(F32)
        k = yb[D:2 * D + 8]
        vta_s[:, t0:t0 + TB] = yb[2 * D:3 * D]
        nq2 = mm(seg, (q[0:D] * q[0:D]).astype(BF16))
        na_s[:, t0:t0 + TB] = -jnp.sqrt(nq2) * MARGIN
        nk2 = mm(seg, (k[0:D] * k[0:D]).astype(BF16))
        for g in range(G):
            qa_s[g, :, t0:t0 + TB] = q[GR * g:GR * g + 80].astype(BF16)
            ka_s[g, t0:t0 + TB, :] = k[GR * g:GR * g + 80].T.astype(BF16)
        return jnp.maximum(kmax, nk2)

    kmax = jnp.zeros((H, TB), F32)
    ys = {0: a_dot(0)}
    for tb in range(NTB):
        if tb + 1 < NTB:
            ys[tb + 1] = a_dot(tb + 1)
        if tb == 1:
            cp_woa.wait()
            wot_s[0:D, :] = woa[...].T
        if tb == 2:
            cp_wob.wait()
            wot_s[D:2 * D, :] = wob[...].T
        kmax = a_post(tb, ys.pop(tb), kmax)
    kn_a = jnp.sqrt(jnp.max(kmax, axis=1, keepdims=True)) * MARGIN

    def a_tiles(tiles, bad, exact):
        r40 = iota((40, 128), 0)
        masks = [jnp.where((r40 >= 9 * j) & (r40 < 9 * j + 9), -1, 0).astype(I32) for j in range(4)]
        r24 = iota((24, 128), 0)
        valid = {}
        for _, _, nk in tiles:
            d = iota((nk, 128), 1) - iota((nk, 128), 0) + (nk - 128)
            valid[nk] = (d >= 0) & (d < WIN)
        us = [(ti, g) for ti in range(len(tiles)) for g in range(G)]
        rows = [[None] * (D // 8) for _ in tiles]
        cs = [na_s[:, pl.ds(q0, 128)] * kn_a for q0, _, _ in tiles]

        def qk(ti, g):
            q0, k0, nk = tiles[ti]
            qi = pltpu.bitcast(qa_s[g, :, pl.ds(q0, 128)], I32)
            w = jnp.concatenate([pltpu.bitcast(qi & masks[j], BF16) for j in range(4)], axis=1)
            return mm(ka_s[g, pl.ds(k0, nk), :], w)

        def pv(ti, g, s, bad):
            q0, k0, nk = tiles[ti]
            rk = iota((24, nk), 0)
            for j in range(4):
                h = 4 * g + j
                a = (DH * h) // 8 * 8
                off = DH * h - a
                rl = 23 if off + DH < 24 else 0
                sj = s[:, 128 * j:128 * j + 128]
                if exact:
                    sj = jnp.where(valid[nk], sj, -jnp.inf)
                    sj = sj - jnp.max(sj, axis=0, keepdims=True)
                else:
                    sj = sj + cs[ti][h:h + 1]
                p = jnp.where(valid[nk], jnp.exp2(sj), 0.0).astype(BF16)
                vw = jnp.where(rk == rl, 1.0, vta_s[a:a + 24, pl.ds(k0, nk)])
                acc = mm(vw, p)
                l = acc[rl:rl + 1]
                bad = jnp.maximum(bad, unsafe_flag(l))
                o = jnp.where((r24 >= off) & (r24 < off + DH), acc * (1.0 / l), 0.0)
                for u in range(3):
                    idx = a // 8 + u
                    piece = o[8 * u:8 * u + 8]
                    rows[ti][idx] = piece if rows[ti][idx] is None else rows[ti][idx] + piece
            return bad

        ss = {0: qk(*us[0])}
        for k, (ti, g) in enumerate(us):
            if k + 1 < len(us):
                ss[k + 1] = qk(*us[k + 1])
            bad = pv(ti, g, ss.pop(k), bad)
            if g == G - 1:
                oa_s[:, pl.ds(tiles[ti][0], 128)] = jnp.concatenate(rows[ti], axis=0).astype(BF16)
        return bad

    def a_attention(exact):
        bad = a_tiles([(0, 0, 128), (128, 0, 256)], jnp.zeros((1, 128), F32), exact)

        def body(t, bad):
            q0 = pl.multiple_of(t * 128, 128)
            k0 = pl.multiple_of(t * 128 - WIN, 128)
            return a_tiles([(q0, k0, WIN + 128)], bad, exact)
        return lax.fori_loop(2, S // 128, body, bad)

    bad_a = a_attention(False)

    @pl.when(jnp.max(bad_a) > 0.0)
    def _a_exact():
        a_attention(True)

    def o_dot(tb):
        t0 = tb * TB
        a = mm(wot_s[0:D, :], oa_s[:, t0:t0 + TB])
        b = mm(wot_s[D:2 * D, :], ob_s[:, t0:t0 + TB].astype(BF16))
        return a, b

    def o_copy(tb):
        return pltpu.make_async_copy(out_v.at[pl.ds(tb * TB, TB), :], out_h.at[pl.ds(tb * TB, TB), :], osem.at[tb])

    ys = {0: o_dot(0)}
    for tb in range(NTB):
        if tb + 1 < NTB:
            ys[tb + 1] = o_dot(tb + 1)
        a, b = ys.pop(tb)
        out_v[tb * TB:(tb + 1) * TB, :] = jnp.concatenate([a, b], axis=0).astype(BF16).T
        o_copy(tb).start()
    for tb in range(NTB):
        o_copy(tb).wait()


@jax.jit
def pallas_concat_heads__sliding_block__grouped_kv_mqa__prompt_kernel(
    A_x: jax.Array,
    A_wqkv: jax.Array,
    A_wo: jax.Array,
    B_x: jax.Array,
    B_wq: jax.Array,
    B_wk: jax.Array,
    B_wv: jax.Array,
    B_wo: jax.Array,
):
    hbm = pl.BlockSpec(memory_space=pltpu.HBM)
    out = pl.pallas_call(
        kernel,
        out_shape=jax.ShapeDtypeStruct((S, 2 * D), BF16),
        in_specs=[hbm] * 8,
        out_specs=hbm,
        scratch_shapes=[
            pltpu.VMEM((D, S), BF16), pltpu.VMEM((D, S), BF16),
            pltpu.VMEM((D, 3 * D), BF16), pltpu.VMEM((D, D), BF16),
            pltpu.VMEM((D, D), BF16), pltpu.VMEM((DH, D), BF16), pltpu.VMEM((DH, D), BF16), pltpu.VMEM((D, D), BF16),
            pltpu.VMEM((D + 64, D), BF16), pltpu.VMEM((3 * D, D), BF16), pltpu.VMEM((2 * D, D), BF16),
            pltpu.VMEM((S, 32), BF16), pltpu.VMEM((24, S), F32), pltpu.VMEM((H, 32, S), BF16),
            pltpu.VMEM((128, 1024), BF16), pltpu.VMEM((D, S), F32),
            pltpu.VMEM((G, S, 80), BF16), pltpu.VMEM((D, S), F32), pltpu.VMEM((G, 80, S), BF16),
            pltpu.VMEM((H, S), F32), pltpu.VMEM((D, S), BF16), pltpu.VMEM((S, 2 * D), BF16),
            pltpu.SemaphoreType.DMA((7,)), pltpu.SemaphoreType.DMA((4,)), pltpu.SemaphoreType.DMA((4,)),
        ],
        compiler_params=pltpu.CompilerParams(vmem_limit_bytes=110 * 1024 * 1024),
    )(A_x.reshape(S, D).T, A_wqkv, A_wo, B_x.reshape(S, D).T, B_wq, B_wk.T, B_wv.T, B_wo)
    return out.reshape(1, S, 2 * D)
```

```python
import math

import jax
import jax.numpy as jnp
from jax import lax
import jax.experimental.pallas as pl
import jax.experimental.pallas.tpu as pltpu

UNR = 2
TPI = 14
LA = 2

S, D, H, DH, WIN = 2048, 576, 32, 18, 256
G = 8
GR = 4 * DH
TB = 512
F32 = jnp.float32
BF16 = jnp.bfloat16
I32 = jnp.int32
SCALE2 = (DH ** -0.5) * math.log2(math.e)
HALF = 0.5 ** 0.5
L_SAFE = 2.0 ** -80
L_HUGE = 2.0 ** 80

NN = ((1,), (0,))


def mm(a, b):
    return lax.dot_general(a, b, (NN, ((), ())), preferred_element_type=F32)


def iota(shape, dim):
    return lax.broadcasted_iota(I32, shape, dim)


def unsafe_flag(l):
    return jnp.where((l >= L_SAFE) & (l <= L_HUGE), 0.0, 1.0)


def kernel(xa_h, wqkv_h, woa_h, xb_h, wq_h, wk_h, wv_h, wob_h, out_h,
           xa, xb, wqkv, woa, wq, wk, wv, wob,
           wbt_s, wat_s, wot_s, kb_s, vtb_s, qb_s, p0_s, ob_s,
           ka_s, vta_s, qa_s, na_s, oa_s, out_v, sems, xsem, osem):
    NTB = S // TB
    def cp(src, dst, sem):
        c = pltpu.make_async_copy(src, dst, sem)
        c.start()
        return c
    cp_wk = cp(wk_h, wk, sems.at[0])
    cp_wv = cp(wv_h, wv, sems.at[1])
    cp_wq = cp(wq_h, wq, sems.at[2])

    def cp_x(tb):
        return cp(xb_h.at[:, pl.ds(tb * TB, TB)], xb.at[:, pl.ds(tb * TB, TB)], xsem.at[tb])
    cp_xb = {}
    late = {}

    SR = 2 * GR
    seg8 = ((iota((8, SR), 1) >= DH * iota((8, SR), 0)) & (iota((8, SR), 1) < DH * iota((8, SR), 0) + DH)).astype(F32)
    r8 = iota((8, TB), 0)

    def norms2(y):
        return mm(seg8, (y * y).astype(BF16))

    def q_post(dst, o, t0, y):
        q = y * SCALE2
        c = -jnp.sqrt(norms2(q)) * HALF
        for u in range(2):
            cu = jnp.where(r8 < 4, pltpu.roll(c, 4, 0) if u else c, 0.0)
            dst[2 * o + u, :, t0:t0 + TB] = jnp.concatenate([q[GR * u:GR * u + GR], cu], axis=0).astype(BF16)
        return c

    wbt_s[D:D + 64, :] = jnp.zeros((64, D), BF16)
    cp_wk.wait()
    cp_xb[0] = cp_x(0)
    wbt_s[D:D + DH, :] = wk[...]
    cp_wv.wait()
    wbt_s[D + 32:D + 32 + DH, :] = wv[...]
    cp_wq.wait()
    cp_xb[1] = cp_x(1)
    wbt_s[0:D, :] = wq[...].T

    jobs = [(tb, o) for tb in range(NTB) for o in range(5)]

    def b_dot(tb, o):
        if o == 0:
            cp_xb[tb].wait()
            if tb == 0:
                cp_xb[2] = cp_x(2)
            if tb == 1:
                cp_xb[3] = cp_x(3)
            if tb == 2:
                late['wqkv'] = cp(wqkv_h, wqkv, sems.at[3])
        rows = SR if o < 4 else 64
        return mm(wbt_s[SR * o:SR * o + rows, :], xb[:, tb * TB:(tb + 1) * TB])

    def b_post(tb, o, y, kmax):
        t0 = tb * TB
        if o < 4:
            q_post(qb_s, o, t0, y)
            return kmax
        kt = y[0:32]
        vtb_s[:, t0:t0 + TB] = jnp.where(iota((24, TB), 0) == DH, 1.0, y[32:56].astype(BF16).astype(F32))
        kb_s[t0:t0 + TB, :] = kt.astype(BF16).T
        return jnp.maximum(kmax, jnp.sum(kt * kt, axis=0, keepdims=True))

    kmax = jnp.zeros((1, TB), F32)
    ys = {0: b_dot(*jobs[0])}
    for n, (tb, o) in enumerate(jobs):
        if n + 1 < len(jobs):
            ys[n + 1] = b_dot(*jobs[n + 1])
        if n == 15:
            late['wqkv'].wait()
        if n >= 15:
            c0, c1 = 384 * (n - 15), min(384 * (n - 14), 3 * D)
            wat_s[c0:c1, :] = wqkv[:, c0:c1].T
        kmax = b_post(tb, o, ys.pop(n), kmax)
    kn = jnp.sqrt(jnp.max(kmax, axis=1, keepdims=True)) * HALF
    kb_s[...] = jnp.where(iota((S, 32), 1) == DH, kn.astype(BF16), kb_s[...])

    cp_xa = cp(xa_h, xa, sems.at[4])
    cp_woa = cp(woa_h, woa, sems.at[5])
    cp_wob = cp(wob_h, wob, sems.at[6])
    QB = 512
    KB = 128
    NS = 1024
    NIT = G * (S // QB)

    def b_w(i, nq=QB, with_c=True):
        sh = (S // nq).bit_length() - 1
        g = i >> sh
        q0 = pl.multiple_of((i & (S // nq - 1)) * nq, nq)
        qi = pltpu.bitcast(qb_s[g, :, pl.ds(q0, nq)], I32)
        r16 = iota((16, nq), 0)
        r8q = iota((8, nq), 0)
        ws = []
        for j in range(4):
            a = 9 * j // 8 * 8
            off = 9 * j - a
            x = qi[a:a + 16]
            if off:
                x = pltpu.roll(x, 16 - off, 0)
            w = jnp.where(r16 < 9, x, 0)
            if with_c:
                cw = pltpu.roll(qi[32:40], 13 - j // 2 - 8, 0)
                cw = lax.shift_right_logical(cw, 16) if j % 2 else cw & 0xFFFF
                w = jnp.concatenate([w[0:8], w[8:16] | jnp.where(r8q == 1, cw, 0)], axis=0)
            ws.append(pltpu.bitcast(w, BF16))
        return jnp.concatenate(ws, axis=1)

    def b_store(g, q0, nq, acc):
        l = acc[DH:DH + 1, :]
        o = jnp.concatenate([acc * (1.0 / l), jnp.zeros((8, 4 * nq), F32)], axis=0)
        r = iota((32, nq), 0)
        rows = [None] * 10
        for j in range(4):
            oj = jnp.where(r < DH, o[:, j * nq:(j + 1) * nq], 0.0)
            if j:
                oj = pltpu.roll(oj, 2 * j, 0)
            for u in range(4):
                piece = oj[8 * u:8 * u + 8]
                idx = 2 * j + u
                rows[idx] = piece if rows[idx] is None else rows[idx] + piece
        ob_s[pl.ds(pl.multiple_of(g * GR, 8), GR), pl.ds(q0, nq)] = jnp.concatenate(rows[0:9], axis=0)
        return l

    units = [(c, n) for n in range(4 * QB // NS) for c in range(S // KB)]
    p0_s[...] = jnp.exp2(mm(kb_s[0:KB, :], b_w(0)[:, 0:NS])).astype(BF16)

    def b_attn(i, bad):
        g = i >> 2
        q0 = pl.multiple_of((i & 3) * QB, QB)
        w = b_w(i)
        accs = [None] * (4 * QB // NS)

        def qk(u, w):
            c, n = u
            return jnp.exp2(mm(kb_s[c * KB:(c + 1) * KB, :], w[:, n * NS:(n + 1) * NS])).astype(BF16)

        ps = {0: p0_s[...]}
        for k, (c, n) in enumerate(units):
            if k + 1 < len(units):
                ps[k + 1] = qk(units[k + 1], w)
            else:
                pn = qk(units[0], b_w(jnp.minimum(i + 1, NIT - 1)))
            r = mm(vtb_s[:, c * KB:(c + 1) * KB], ps.pop(k))
            accs[n] = r if accs[n] is None else accs[n] + r
        p0_s[...] = pn
        l = b_store(g, q0, QB, jnp.concatenate(accs, axis=1))
        for j in range(4):
            bad = jnp.maximum(bad, unsafe_flag(l[:, j * QB:(j + 1) * QB]))
        return bad
    bad_b = lax.fori_loop(0, NIT, b_attn, jnp.zeros((1, QB), F32), unroll=UNR)

    @pl.when(jnp.max(bad_b) > 0.0)
    def _b_exact():
        def body(i, carry):
            g = i // (S // 128)
            q0 = pl.multiple_of((i % (S // 128)) * 128, 128)
            accs = []
            xw = b_w(i, 128, False)
            for j in range(4):
                w = xw[:, 128 * j:128 * j + 128]

                def scores(c):
                    return mm(kb_s[pl.ds(pl.multiple_of(c * 512, 512), 512), :], w)

                def max_step(c, m):
                    return jnp.maximum(m, jnp.max(scores(c), axis=0, keepdims=True))
                m = lax.fori_loop(0, S // 512, max_step, jnp.full((1, 128), -jnp.inf, F32))

                def acc_step(c, acc):
                    p = jnp.exp2(scores(c) - m).astype(BF16)
                    return acc + mm(vtb_s[:, pl.ds(pl.multiple_of(c * 512, 512), 512)], p)
                accs.append(lax.fori_loop(0, S // 512, acc_step, jnp.zeros((24, 128), F32)))
            b_store(g, q0, 128, jnp.concatenate(accs, axis=1))
            return carry
        lax.fori_loop(0, G * (S // 128), body, 0)

    cp_xa.wait()
    jobs = [(tb, o) for tb in range(NTB) for o in range(12)]

    def a_dot(tb, o):
        return mm(wat_s[SR * o:SR * o + SR, :], xa[:, tb * TB:(tb + 1) * TB])

    def a_post(tb, o, y):
        t0 = tb * TB
        if o < 4:
            na_s[8 * o:8 * o + 8, t0:t0 + TB] = q_post(qa_s, o, t0, y)
        elif o < 8:
            kmax[o - 4] = jnp.maximum(kmax[o - 4], norms2(y))
            for u in range(2):
                kg = jnp.concatenate([y[GR * u:GR * u + GR], jnp.zeros((8, TB), F32)], axis=0)
                ka_s[2 * (o - 4) + u, t0:t0 + TB, :] = kg.astype(BF16).T
        else:
            vta_s[SR * (o - 8):SR * (o - 7), t0:t0 + TB] = y.astype(BF16).astype(F32)

    kmax = [jnp.zeros((8, TB), F32) for _ in range(4)]
    ys = {0: a_dot(*jobs[0])}
    for n, (tb, o) in enumerate(jobs):
        if n + 1 < len(jobs):
            ys[n + 1] = a_dot(*jobs[n + 1])
        if n == 12:
            cp_woa.wait()
        if n == 24:
            cp_wob.wait()
        if 12 <= n < 15 or 24 <= n < 27:
            src, base, m = (woa, 0, n - 12) if n < 24 else (wob, D, n - 24)
            c0, c1 = 256 * m, min(256 * (m + 1), D)
            wot_s[base + c0:base + c1, :] = src[:, c0:c1].T
        a_post(tb, o, ys.pop(n))
    kn_a = jnp.sqrt(jnp.max(jnp.concatenate(kmax, axis=0), axis=1, keepdims=True)) * HALF

    def a_tiles(tiles, bad, exact):
        r40 = iota((40, 128), 0)
        masks = [jnp.where((r40 >= 9 * j) & (r40 < 9 * j + 9), -1, 0).astype(I32) for j in range(4)]
        r24 = iota((24, 128), 0)
        rr, cc = iota((128, 128), 0), iota((128, 128), 1)
        d = cc - rr
        valid = {0: d + WIN < WIN, 2: (d >= 0) & (d < WIN)}
        rows = [[None] * (D // 8) for _ in tiles]
        cs = [na_s[:, pl.ds(q0, 128)] * kn_a for q0, _ in tiles]
        ws = {}

        def weights(ti, g):
            if (ti, g) not in ws:
                qi = pltpu.bitcast(qa_s[g, :, pl.ds(tiles[ti][0], 128)], I32)
                ws[ti, g] = jnp.concatenate([pltpu.bitcast(qi & masks[j], BF16) for j in range(4)], axis=1)
            return ws[ti, g]

        def scores(ti, g, kt):
            return mm(ka_s[g, pl.ds(tiles[ti][0] - WIN + 128 * kt, 128), :], weights(ti, g))

        def probs(g, kt, s, shift):
            ps = []
            for j in range(4):
                e = jnp.exp2(s[:, 128 * j:128 * j + 128] + shift[j])
                ps.append((jnp.where(valid[kt], e, 0.0) if kt in valid else e).astype(BF16))
            return ps

        accs = {}

        def pv(ti, g, kt, ps, bad):
            q0, kts = tiles[ti]
            for j in range(4):
                h = 4 * g + j
                a = (DH * h) // 8 * 8
                off = DH * h - a
                rl = 23 if off + DH < 24 else 0
                vw = jnp.where(r24 == rl, 1.0, vta_s[a:a + 24, pl.ds(q0 - WIN + 128 * kt, 128)])
                r = mm(vw, ps[j])
                accs[j] = r if kt == kts[0] else accs[j] + r
                if kt == kts[-1]:
                    l = accs[j][rl:rl + 1]
                    bad = jnp.maximum(bad, unsafe_flag(l))
                    o = jnp.where((r24 >= off) & (r24 < off + DH), accs[j] * (1.0 / l), 0.0)
                    for u in range(3):
                        idx = a // 8 + u
                        piece = o[8 * u:8 * u + 8]
                        rows[ti][idx] = piece if rows[ti][idx] is None else rows[ti][idx] + piece
            if g == G - 1 and kt == kts[-1]:
                oa_s[:, pl.ds(q0, 128)] = jnp.concatenate(rows[ti], axis=0).astype(BF16)
            return bad

        us = [(ti, g, kt) for ti, (_, kts) in enumerate(tiles) for g in range(G) for kt in kts]
        if exact:
            for ti, (_, kts) in enumerate(tiles):
                for g in range(G):
                    ss = {kt: scores(ti, g, kt) for kt in kts}
                    shift = []
                    for j in range(4):
                        m = None
                        for kt in kts:
                            sj = ss[kt][:, 128 * j:128 * j + 128]
                            mk = jnp.max(jnp.where(valid[kt], sj, -jnp.inf) if kt in valid else sj, axis=0, keepdims=True)
                            m = mk if m is None else jnp.maximum(m, mk)
                        shift.append(-m)
                    for kt in kts:
                        bad = pv(ti, g, kt, probs(g, kt, ss[kt], shift), bad)
            return bad

        def qk(ti, g, kt):
            return probs(g, kt, scores(ti, g, kt), [cs[ti][4 * g + j:4 * g + j + 1] for j in range(4)])
        pend = {k: qk(*us[k]) for k in range(LA)}
        for k, u in enumerate(us):
            if k + LA < len(us):
                pend[k + LA] = qk(*us[k + LA])
            bad = pv(*u, pend.pop(k), bad)
        return bad

    def a_attention(exact):
        tpi = 1 if exact else TPI
        first = [(0, (2,)), (128, (1, 2))]
        bad = a_tiles(first, jnp.zeros((1, 128), F32), exact)

        def body(i, bad):
            tiles = []
            for u in range(tpi):
                t = 2 + i * tpi + u
                tiles.append((pl.multiple_of(t * 128, 128), (0, 1, 2)))
            return a_tiles(tiles, bad, exact)
        return lax.fori_loop(0, (S // 128 - 2) // tpi, body, bad)

    bad_a = a_attention(False)

    @pl.when(jnp.max(bad_a) > 0.0)
    def _a_exact():
        a_attention(True)

    jobs = [(tb, o) for tb in range(NTB) for o in range(9)]

    def o_dot(tb, o):
        t0 = tb * TB
        r0 = 128 * o
        if r0 + 128 <= D:
            return mm(wot_s[r0:r0 + 128, :], oa_s[:, t0:t0 + TB])
        if r0 >= D:
            return mm(wot_s[r0:r0 + 128, :], ob_s[:, t0:t0 + TB].astype(BF16))
        return jnp.concatenate([mm(wot_s[r0:D, :], oa_s[:, t0:t0 + TB]), mm(wot_s[D:r0 + 128, :], ob_s[:, t0:t0 + TB].astype(BF16))], axis=0)

    parts = [(128 * i, 128 * i + 128) for i in range(9)]

    def o_copy(tb, p):
        c0, c1 = parts[p]
        return pltpu.make_async_copy(out_v.at[pl.ds(tb * TB, TB), pl.ds(c0, c1 - c0)],
                                     out_h.at[pl.ds(tb * TB, TB), pl.ds(c0, c1 - c0)], osem.at[tb * 9 + p])

    ys = {0: o_dot(*jobs[0])}
    for n, (tb, o) in enumerate(jobs):
        if n + 1 < len(jobs):
            ys[n + 1] = o_dot(*jobs[n + 1])
        out_v[tb * TB:(tb + 1) * TB, 128 * o:128 * o + 128] = ys.pop(n).astype(BF16).T
        for p, (c0, c1) in enumerate(parts):
            if c1 == 128 * o + 128:
                o_copy(tb, p).start()
    for tb in range(NTB):
        for p in range(len(parts)):
            o_copy(tb, p).wait()


@jax.jit
def pallas_concat_heads__sliding_block__grouped_kv_mqa__prompt_kernel(
    A_x: jax.Array,
    A_wqkv: jax.Array,
    A_wo: jax.Array,
    B_x: jax.Array,
    B_wq: jax.Array,
    B_wk: jax.Array,
    B_wv: jax.Array,
    B_wo: jax.Array,
):
    hbm = pl.BlockSpec(memory_space=pltpu.HBM)
    out = pl.pallas_call(
        kernel,
        out_shape=jax.ShapeDtypeStruct((S, 2 * D), BF16),
        in_specs=[hbm] * 8,
        out_specs=hbm,
        scratch_shapes=[
            pltpu.VMEM((D, S), BF16), pltpu.VMEM((D, S), BF16),
            pltpu.VMEM((D, 3 * D), BF16), pltpu.VMEM((D, D), BF16),
            pltpu.VMEM((D, D), BF16), pltpu.VMEM((DH, D), BF16), pltpu.VMEM((DH, D), BF16), pltpu.VMEM((D, D), BF16),
            pltpu.VMEM((D + 64, D), BF16), pltpu.VMEM((3 * D, D), BF16), pltpu.VMEM((2 * D, D), BF16),
            pltpu.VMEM((S, 32), BF16), pltpu.VMEM((24, S), F32), pltpu.VMEM((G, 80, S), BF16),
            pltpu.VMEM((128, 1024), BF16), pltpu.VMEM((D, S), F32),
            pltpu.VMEM((G, S, 80), BF16), pltpu.VMEM((D, S), F32), pltpu.VMEM((G, 80, S), BF16),
            pltpu.VMEM((H, S), F32), pltpu.VMEM((D, S), BF16), pltpu.VMEM((S, 2 * D), BF16),
            pltpu.SemaphoreType.DMA((8,)), pltpu.SemaphoreType.DMA((4,)), pltpu.SemaphoreType.DMA((36,)),
        ],
        compiler_params=pltpu.CompilerParams(vmem_limit_bytes=110 * 1024 * 1024, flags={'XLA_TPU_EVENLY_DISTRIBUTE_CRITICAL_NODES': True}),
    )(A_x.reshape(S, D).T, A_wqkv, A_wo, B_x.reshape(S, D).T, B_wq, B_wk.T, B_wv.T, B_wo)
    return out.reshape(1, S, 2 * D)
```
